```python
import jax
import jax.numpy as jnp

def _softmax(x, axis=-1):
    return jax.nn.softmax(x, axis=axis)

def _gelu(x):
    return jax.nn.gelu(x, approximate=True)

def _silu(x):
    return jax.nn.silu(x)

def _sigmoid(x):
    return jax.nn.sigmoid(x)

def _layernorm(x, axis=-1, eps=1e-05):
    m = jnp.mean(x, axis=axis, keepdims=True)
    v = jnp.var(x, axis=axis, keepdims=True)
    return (x - m) / jnp.sqrt(v + eps)

def _scatter_add(tgt, idx, src, axis=0):
    return tgt.at[idx].add(src)

def _segment_sum(src, seg, n):
    return jax.ops.segment_sum(src, seg, n)

class _Rng:

    def __init__(self, key):
        self._k = key

    def _next(self):
        self._k, sub = jax.random.split(self._k)
        return sub

    def normal(self, shape):
        return jax.random.normal(self._next(), shape, dtype=jnp.bfloat16)

    def randint(self, lo, hi, shape):
        return jax.random.randint(self._next(), shape, lo, hi, dtype=jnp.int32)

    def uniform(self, shape, lo=0.0, hi=1.0):
        return jax.random.uniform(self._next(), shape, jnp.bfloat16, lo, hi)

    def permutation(self, n):
        return jax.random.permutation(self._next(), n)
kernel_name = 'adaLN_cond__ssm_conv_h3__glu_gated_reglu__prompt'

def setup_inputs():
    _rng = _Rng(jax.random.key(int.from_bytes(__import__("os").urandom(4), "little")))
    _w = lambda a: (lambda t: t.astype(jnp.bfloat16) if jnp.issubdtype(t.dtype, jnp.floating) else t)(jnp.asarray(a))

    def _A_setup():
        B, S, D = (1, 2048, 640)
        ks = 4
        return {'q': _w((lambda *s: _rng.normal(s) * 0.05)(B, S, D)), 'k': _w((lambda *s: _rng.normal(s) * 0.05)(B, S, D)), 'v': _w((lambda *s: _rng.normal(s) * 0.05)(B, S, D)), 'shift_k': _w((lambda *s: _rng.normal(s) * 0.05)(D, ks) * 0.5), 'ssm_k': _w((lambda *s: _rng.normal(s) * 0.05)(D, S) * (1.0 / S ** 0.5)), 'ssm_D': _w((lambda *s: _rng.normal(s) * 0.05)(D))}
    _A_in = _A_setup()

    def _B_setup():
        B, S, D, F = (1, 2048, 640, 1536)
        return {'x': _w((lambda *s: _rng.normal(s) * 0.05)(B, S, D)), 'W_gate': _w((lambda *s: _rng.normal(s) * 0.05)(D, F) * (2.0 / D) ** 0.5), 'W_up': _w((lambda *s: _rng.normal(s) * 0.05)(D, F) * (2.0 / D) ** 0.5), 'W_down': _w((lambda *s: _rng.normal(s) * 0.05)(F, D) * (1.0 / F) ** 0.5)}
    _B_in = _B_setup()
    return {'A_q': _A_in['q'], 'A_k': _A_in['k'], 'A_v': _A_in['v'], 'A_shift_k': _A_in['shift_k'], 'A_ssm_k': _A_in['ssm_k'], 'A_ssm_D': _A_in['ssm_D'], 'B_x': _B_in['x'], 'B_W_gate': _B_in['W_gate'], 'B_W_up': _B_in['W_up'], 'B_W_down': _B_in['W_down'], 'c': _w((lambda *s: _rng.normal(s) * 0.05)(1, 640)), 'w_mod': _w((lambda *s: _rng.normal(s) * 0.05)(640, 6 * 640) * 640 ** (-0.5))}

def reference(A_q, A_k, A_v, A_shift_k, A_ssm_k, A_ssm_D, B_x, B_W_gate, B_W_up, B_W_down, c, w_mod):

    def _A_ref(q, k, v, shift_k, ssm_k, ssm_D):
        B, S, D = q.shape
        ks = shift_k.shape[-1]
        k_pad = jnp.pad(k, ((0, 0), (ks - 1, 0), (0, 0)))
        k_shift = jnp.zeros_like(k)
        for t in range(ks):
            k_shift = k_shift + k_pad[:, t:t + S, :] * shift_k[:, ks - 1 - t][None, None, :]
        kv = k_shift * v
        L = 2 * S
        kv_pad = jnp.pad(kv, ((0, 0), (0, S), (0, 0)))
        kf_pad = jnp.pad(ssm_k, ((0, 0), (0, S)))
        kv_f = (lambda x, axes=(-2, -1): jnp.fft.rfft2(x.astype(jnp.float32), axes=axes))(kv_pad[:, None, :, :], axes=(1, 2))
        kf_f = (lambda x, axes=(-2, -1): jnp.fft.rfft2(x.astype(jnp.float32), axes=axes))(kf_pad[:, None, :], axes=(1, 2))
        kf_f = (lambda x, *d: x.transpose(*d))(kf_f, 1, 2, 0)
        y_f = kv_f * kf_f[None, :, :, :]
        y = (lambda x, s, axes=(-2, -1): jnp.fft.irfft2(x, s=s, axes=axes).astype(jnp.bfloat16))(y_f, (1, L), axes=(1, 2))[:, 0, :S, :]
        y = y + kv * ssm_D[None, None, :]
        return q * y

    def _B_ref(x, W_gate, W_up, W_down):
        gate = jnp.einsum('bsd,df->bsf', x, W_gate)
        up = jnp.einsum('bsd,df->bsf', x, W_up)
        gate = gate * (lambda x, dt: x.astype(dt))(gate > 0, gate.dtype)
        h = gate * up
        return jnp.einsum('bsf,fd->bsd', h, W_down)
    x = A_q
    mod = (_silu(c) @ w_mod).reshape(c.shape[0], 6, 1, -1)
    sa, ca, ga, sb, cb, gb = (mod[:, 0].copy(), mod[:, 1].copy(), mod[:, 2].copy(), mod[:, 3].copy(), mod[:, 4].copy(), mod[:, 5].copy())
    h = _layernorm(x, axis=-1) * (1 + ca) + sa
    x = x + ga * _A_ref(h, A_k, A_v, A_shift_k, A_ssm_k, A_ssm_D)
    h = _layernorm(x, axis=-1) * (1 + cb) + sb
    x = x + gb * _B_ref(h, B_W_gate, B_W_up, B_W_down)
    return x
```

```python
import functools, os
import numpy as np
import jax
import jax.numpy as jnp
import jax.experimental.pallas as pl
import jax.experimental.pallas.tpu as pltpu

S, D, F = 2048, 640, 1536
C = 128
NC = S // C
KS = 4
EPS = 1e-5
MB = int(os.environ.get("MB", "256"))
NB = S // MB
CPB = MB // C
FG = int(os.environ.get("FG", "256"))
NG = F // FG
FT = int(os.environ.get("FT", "8"))
LT = int(os.environ.get("LT", "640"))
ABL = os.environ.get("ABL", "")
BIG = int(os.environ.get("BIG", "0"))
DYN = int(os.environ.get("DYN", "0"))
DEP = int(os.environ.get("DEP", "0"))
IL = int(os.environ.get("IL", "2"))
M3 = int(os.environ.get("M3", "1"))
PAIR = int(os.environ.get("PAIR", "1"))
JREV = int(os.environ.get("JREV", "0"))
ORD = int(os.environ.get("ORD", "0"))
DSPLIT = int(os.environ.get("DSPLIT", "0"))
LNR = int(os.environ.get("LNR", "0"))
PP = int(os.environ.get("PP", "6"))
STOP = int(os.environ.get("STOP", "99"))
TAIL = int(os.environ.get("TAIL", "1"))
GW = [int(a) for a in os.environ.get("GW", "0,2,4").split(",")] + [NG]
SPM = int(os.environ.get("SPM", "0"))
RST = int(os.environ.get("RST", "1"))
BB = int(os.environ.get("BB", "0"))
NOBAR = int(os.environ.get("NOBAR", "1"))
DNP = int(os.environ.get("DNP", "0"))
NSPL = int(os.environ.get("NSPL", "2"))
TOKALL = int(os.environ.get("TOKALL", "0"))
LAG = int(os.environ.get("LAG", "2"))
NP = 3 if M3 else 2

def _dft_consts():
    j = np.arange(C, dtype=np.float64)[:, None]
    n = np.arange(C, dtype=np.float64)[None, :]
    ang = np.pi * (2 * j + 1) * n / (2 * C) * np.where(j % 2 == 0, 1.0, -1.0)
    wf = np.concatenate([np.cos(ang), -np.sin(ang)], axis=0)
    wi = np.concatenate([np.cos(ang).T, -np.sin(ang).T], axis=1) / C
    return wf.astype(np.float32), wi.astype(np.float32)

_WF, _WI = _dft_consts()
if IL:
    _perm = np.concatenate([np.concatenate([np.arange(f0, f0 + FT), C + np.arange(f0, f0 + FT)]) for f0 in range(0, C, FT)])
    _WI = _WI[:, _perm]

def _ln(x):
    m = jnp.mean(x, axis=-1, keepdims=True)
    xc = x - m
    v = jnp.mean(xc * xc, axis=-1, keepdims=True)
    return xc * jax.lax.rsqrt(v + EPS)

def kernel(x_hbm, k_hbm, v_hbm, sk_hbm, ssmk_hbm, sd_hbm, wg_hbm, wu_hbm, wd_hbm, c_hbm, wm_hbm,
           wf_hbm, wi_hbm, o_hbm,
           x_v, k_v, v_v, sk_v, ssmk_v, sd_v, wg_v, wu_v, wd_v, c_v, wm_v, wf_v, wi_v, o_v,
           g_scr, xs_scr, kr_scr, y_scr, yy_scr, x1_scr, h2_scr, hh_scr, mod_scr, taps_scr, sems, osems):
    f32, bf16 = jnp.float32, jnp.bfloat16
    if BIG:
        g_big, x_big = g_scr, xs_scr
        g_scr = [g_big.at[m] for m in range(NC)]
        xs_scr = [x_big.at[m] for m in range(NC)]

    dmas = {}
    order = []
    def add(name, src, dst):
        dmas[name] = pltpu.make_async_copy(src, dst, sems.at[len(order)])
        order.append(name)
    def rows(b): return pl.ds(b * MB, MB)
    def add_blk(b):
        add(("k", b), k_hbm.at[rows(b), :], k_v.at[rows(b), :])
        add(("v", b), v_hbm.at[rows(b), :], v_v.at[rows(b), :])
        add(("ssmk", b), ssmk_hbm.at[:, rows(b)], ssmk_v.at[:, rows(b)])
    def add_wm(i):
        add(("wm", i), wm_hbm.at[:, pl.ds(i * D, D)], wm_v.at[:, pl.ds(i * D, D)])
    def add_x(b):
        add(("x", b), x_hbm.at[rows(b), :], x_v.at[rows(b), :])
    add("wf", wf_hbm, wf_v); add("sk", sk_hbm, sk_v); add("sd", sd_hbm, sd_v)
    wm_after = [int(a) for a in os.environ.get("WMPOS", "4,5,5,6,6").split(",")]
    for b in range(NB):
        add_blk(b)
        if b == 0:
            add("wi", wi_hbm, wi_v); add("c", c_hbm, c_v)
        for i in range(5):
            if wm_after[i] == b:
                add_wm(i)
        if b == max(wm_after):
            add_x(0)
    for q in range(len(GW) - 1):
        cs = pl.ds(GW[q] * FG, (GW[q + 1] - GW[q]) * FG)
        add(("wg", q), wg_hbm.at[:, cs], wg_v.at[:, cs])
        add(("wu", q), wu_hbm.at[:, cs], wu_v.at[:, cs])
    add_x(1)
    if LAG == 2:
        add_x(2)
    add("wd", wd_hbm, wd_v)
    add_wm(5)
    for b in range(2 if LAG == 1 else 3, NB):
        add_x(b)
    if STOP < 0:
        order[:] = order[:order.index(("wg", 0))]
    elif STOP == 0:
        order[:] = order[:order.index("wd")]
    elif STOP < 6:
        order[:] = order[:order.index(("x", STOP + 1)) + 1]
    for name in order:
        dmas[name].start()
    waited = set()
    def wait(*names):
        for n in names:
            if n not in waited:
                dmas[n].wait()
                waited.add(n)

    def setup():
        taps_scr[0:KS, :] = sk_v[...].astype(f32)
        taps_scr[8:9, :] = sd_v[...].astype(f32)

    def mod_piece(i):
        cc = c_v[...].astype(f32)
        sc = (cc * jax.nn.sigmoid(cc)).astype(bf16)
        sc8 = jnp.broadcast_to(sc, (16, D))
        r = jnp.dot(sc8, wm_v[:, i * D:(i + 1) * D], preferred_element_type=f32)[0:1, :]
        if i in (1, 4):
            r = r + 1.0
        mod_scr[i:i + 1, :] = r

    def k_spec(m):
        km = jax.lax.dot_general(wf_v[...], ssmk_v[:, m * C:(m + 1) * C], (((1,), (1,)), ((), ())),
                                 preferred_element_type=f32)
        kre, kim = km[:C], km[C:]
        if m == 0:
            ga_, gb_ = kre, kim
        else:
            kp = kr_scr[m - 1]
            ga_ = kre - kp[C:2 * C, :]
            gb_ = kim + kp[0:C, :]
        g_scr[m][0:C, :] = ga_
        g_scr[m][C:2 * C, :] = gb_
        if M3:
            g_scr[m][2 * C:3 * C, :] = ga_ + gb_
        if m < NC - 1:
            kp = kr_scr[m]
            kp[0:C, :] = kre
            kp[C:2 * C, :] = kim

    def x_spec(i):
        r0 = i * C
        if i == 0:
            kw = jnp.concatenate([jnp.zeros((16, D), f32), k_v[0:C, :].astype(f32)], axis=0)
        else:
            kw = k_v[r0 - 16:r0 + C, :].astype(f32)
        ks = None
        for s in range(KS):
            term = kw[16 - s:16 - s + C, :] * taps_scr[s:s + 1, :]
            ks = term if ks is None else ks + term
        kv = ks * v_v[r0:r0 + C, :].astype(f32)
        yy_scr[i][...] = kv * taps_scr[8:9, :]
        xm = jnp.dot(wf_v[...], kv.astype(bf16), preferred_element_type=f32)
        if M3:
            xc_, xd_ = xm[:C], xm[C:]
            xs_scr[i][0:C, :] = xc_
            xs_scr[i][C:2 * C, :] = xd_ - xc_
            xs_scr[i][2 * C:3 * C, :] = xc_ + xd_
        else:
            xs_scr[i][...] = xm

    dep = [None]
    def accum_tile(i, f0):
        if DYN:
            z = pl.multiple_of(z_ref[i], 8)
            rre = pl.ds(z + f0, FT); rim = pl.ds(z + C + f0, FT)
        else:
            rre = pl.ds(f0, FT); rim = pl.ds(C + f0, FT)
        for l0 in range(0, D, LT):
            are = aim = None
            for j in range(i + 1):
                gre = g_scr[i - j][rre, l0:l0 + LT]
                gim = g_scr[i - j][rim, l0:l0 + LT]
                xre = xs_scr[j][rre, l0:l0 + LT]
                xim = xs_scr[j][rim, l0:l0 + LT]
                pre = gre * xre - gim * xim
                pim = gre * xim + gim * xre
                if are is None and DEP and dep[0] is not None:
                    pre = jnp.where(tmask, pre, dep[0][1])
                    pim = jnp.where(tmask, pim, dep[0][0])
                are = pre if are is None else are + pre
                aim = pim if aim is None else aim + pim
            if DEP:
                dep[0] = (are, aim)
            if IL == 2:
                y_scr[i][2 * f0:2 * f0 + 2 * FT, l0:l0 + LT] = jnp.concatenate([are, aim], axis=0).astype(bf16)
            else:
                o0, o1 = (2 * f0, 2 * f0 + FT) if IL else (f0, C + f0)
                y_scr[i][o0:o0 + FT, l0:l0 + LT] = are.astype(bf16)
                y_scr[i][o1:o1 + FT, l0:l0 + LT] = aim.astype(bf16)

    def accum_pair_parts(p, f0, l0, nsplit):
        i0, i1 = 2 * p, 2 * p + 1
        T = 8
        def ld(ref):
            return [ref[q * C + f0:q * C + f0 + T, l0:l0 + 128] for q in range(NP)]
        gc = {}
        def G(m):
            if m not in gc:
                gc[m] = ld(g_scr[m])
            return gc[m]
        acc = {i0: None, i1: None}
        order = list(range(i1 + 1)) if JREV == 0 else list(range(i1, -1, -1))
        nsplit = min(nsplit, len(order))
        def part(k):
            js = order[(len(order) * k) // nsplit:(len(order) * (k + 1)) // nsplit]
            for j in js:
                xj = ld(xs_scr[j])
                for i in (i0, i1):
                    if j > i:
                        continue
                    g = G(i - j)
                    if M3:
                        pr = [xj[0] * g[2], g[0] * xj[1], g[1] * xj[2]]
                    else:
                        pr = [g[0] * xj[0] - g[1] * xj[1], g[0] * xj[1] + g[1] * xj[0]]
                    acc[i] = pr if acc[i] is None else [a + b for a, b in zip(acc[i], pr)]
            if k < nsplit - 1:
                t = None
                for i in (i0, i1):
                    if acc[i] is not None:
                        for a in (acc[i] if TOKALL else acc[i][:1]):
                            bt = pltpu.bitcast(a, jnp.int32)
                            t = bt if t is None else t | bt
                return t
            if M3:
                res = [(acc[i][0] - acc[i][2], acc[i][0] + acc[i][1]) for i in (i0, i1)]
            else:
                res = [tuple(acc[i]) for i in (i0, i1)]
            re = jnp.concatenate([res[0][0], res[1][0]], axis=1)
            im = jnp.concatenate([res[0][1], res[1][1]], axis=1)
            yv = jnp.concatenate([re, im], axis=0).astype(bf16)
            y_scr[p][2 * f0:2 * f0 + 2 * T, 2 * l0:2 * l0 + 256] = yv
            return token(yv)
        return [functools.partial(part, k) for k in range(nsplit)]

    def accum_pair_tile(p, f0, l0):
        return accum_pair_parts(p, f0, l0, 1)[0]()

    def accum(i):
        if PAIR:
            if i % 2 == 1:
                for f0 in range(0, C, 8):
                    for l0 in range(0, D, 128):
                        accum_pair_tile(i // 2, f0, l0)
            return
        for f0 in range(0, C, FT):
            accum_tile(i, f0)

    def inv(i):
        if PAIR:
            if i % 2 == 1:
                r = jnp.dot(wi_v[...], y_scr[i // 2][...], preferred_element_type=f32)
                for q, ii in enumerate((i - 1, i)):
                    rr = jnp.concatenate([r[:, 256 * t + 128 * q:256 * t + 128 * q + 128] for t in range(D // 128)], axis=1)
                    yy_scr[ii][...] = yy_scr[ii][...] + rr
            return
        yy_scr[i][...] = yy_scr[i][...] + jnp.dot(wi_v[...], y_scr[i][...], preferred_element_type=f32)

    def conv_out(i):
        r0 = i * C
        x = x_v[r0:r0 + C, :].astype(f32)
        if "L" in ABL:
            b = r0 // MB; lr = r0 % MB
            x1_scr[b][lr:lr + C, :] = x + yy_scr[i][...]
            h2_scr[b][lr:lr + C, :] = x_v[r0:r0 + C, :]
            return
        h = _ln(x) * mod_scr[1:2, :] + mod_scr[0:1, :]
        x1 = x + mod_scr[2:3, :] * (h * yy_scr[i][...])
        b = r0 // MB
        lr = r0 % MB
        x1_scr[b][lr:lr + C, :] = x1
        h2_scr[b][lr:lr + C, :] = (_ln(x1) * mod_scr[4:5, :] + mod_scr[3:4, :]).astype(bf16)

    i32 = jnp.int32
    def token(val_bf16):
        bits = pltpu.bitcast(val_bf16, i32)
        t = None
        for q in range(bits.shape[1] // 128):
            p = bits[:, q * 128:(q + 1) * 128]
            t = p if t is None else t | p
        return t

    def attach(w, toks):
        if not toks:
            return w
        m = jnp.abs(wf_v[0:16, :].astype(f32))[0:8] <= 2.0
        K, N = w.shape
        byrow = {}
        for r16, ct, t in toks:
            byrow.setdefault(r16, []).append((ct, t))
        outr = []
        prev = 0
        for r16 in sorted(byrow):
            r0 = r16 * 16
            if r0 > prev:
                outr.append(w[prev:r0])
            cols = []
            pc = 0
            for ct, t in sorted(byrow[r16], key=lambda a: a[0]):
                c0 = ct * 128
                if c0 > pc:
                    cols.append(w[r0:r0 + 16, pc:c0])
                wb = pltpu.bitcast(w[r0:r0 + 16, c0:c0 + 128], i32)
                cols.append(pltpu.bitcast(jnp.where(m, wb, t), bf16))
                pc = c0 + 128
            if pc < N:
                cols.append(w[r0:r0 + 16, pc:N])
            outr.append(cols[0] if len(cols) == 1 else jnp.concatenate(cols, axis=1))
            prev = r0 + 16
        if prev < K:
            outr.append(w[prev:K])
        return jnp.concatenate(outr, axis=0)

    rowctr = [0]
    def spread(pieces, K, N):
        nk, nn = K // 128, N // 128
        if SPM == 0:
            pos = [(kt, ct) for kt in range(nk) for ct in range(nn)]
        else:
            pos = [(kt, ct) for ct in range(nn) for kt in range(nk)]
        toks = []
        n = len(pieces)
        used = set()
        for q, p in enumerate(pieces):
            idx = (q * len(pos)) // n
            kt, ct = pos[idx]
            r = rowctr[0] % 8
            while (kt * 8 + r, ct) in used:
                r = (r + 1) % 8
            rowctr[0] += RST
            used.add((kt * 8 + r, ct))
            toks.append((kt * 8 + r, ct, p()))
        return toks

    def gu(b, g, pg=(), pu=()):
        h = h2_scr[b][...]
        nt = FG // 128
        wg_ = attach(wg_v[:, g * FG:(g + 1) * FG], spread(pg, D, FG))
        gt = jnp.dot(h, wg_, preferred_element_type=f32)
        wu_ = attach(wu_v[:, g * FG:(g + 1) * FG], spread(pu, D, FG))
        ut = jnp.dot(h, wu_, preferred_element_type=f32)
        hh_scr[b][:, g * FG:(g + 1) * FG] = (jnp.maximum(gt, 0.0) * ut).astype(bf16)

    def down_tile(b, n, pd=()):
        wd_ = attach(wd_v[:, n * 128:(n + 1) * 128], spread(pd, F, 128))
        out = jnp.dot(hh_scr[b][...], wd_, preferred_element_type=f32)
        cs = slice(n * 128, (n + 1) * 128)
        o_v[b * MB:(b + 1) * MB, cs] = (x1_scr[b][:, cs] + mod_scr[5:6, cs] * out).astype(o_v.dtype)

    def down(b):
        if DSPLIT:
            for n in range(D // 128):
                down_tile(b, n)
            return
        out = jnp.dot(hh_scr[b][...], wd_v[...], preferred_element_type=f32)
        o_v[b * MB:(b + 1) * MB, :] = (x1_scr[b][...] + mod_scr[5:6, :] * out).astype(o_v.dtype)

    def conv_out_piece(r0, R):
        def f():
            i = r0 // C
            lc = r0 % C
            x = x_v[r0:r0 + R, :].astype(f32)
            if "L" in ABL:
                b = r0 // MB; lr = r0 % MB
                x1_scr[b][lr:lr + R, :] = x
                h2_scr[b][lr:lr + R, :] = x_v[r0:r0 + R, :]
                return token(x_v[r0:r0 + 16, 0:128])
            h = _ln(x) * mod_scr[1:2, :] + mod_scr[0:1, :]
            x1 = x + mod_scr[2:3, :] * (h * yy_scr[i][lc:lc + R, :])
            b = r0 // MB
            lr = r0 % MB
            x1_scr[b][lr:lr + R, :] = x1
            h2 = (_ln(x1) * mod_scr[4:5, :] + mod_scr[3:4, :]).astype(bf16)
            h2_scr[b][lr:lr + R, :] = h2
            t = None
            for q in range(R // 16):
                tt = token(h2[q * 16:(q + 1) * 16])
                t = tt if t is None else t | tt
            return t
        return f

    def ln_pieces(b):
        if LNR == 0:
            for i in chunks(b):
                conv_out(i)
            return []
        return [conv_out_piece(r0, LNR) for r0 in range(b * MB, (b + 1) * MB, LNR)]

    def acc_pieces(b):
        ps = []
        for p in range(b * CPB // 2, (b + 1) * CPB // 2):
            for f0 in range(0, C, 8):
                for l0 in range(0, D, 128):
                    ps += accum_pair_parts(p, f0, l0, NSPL)
        return ps

    odma = [pltpu.make_async_copy(o_v.at[rows(b), :], o_hbm.at[rows(b), :], osems.at[b]) for b in range(NB - 1 if TAIL else NB)]
    def chunks(b): return range(b * CPB, (b + 1) * CPB)

    def region(dots, pieces):
        n = len(dots)
        for q, d in enumerate(dots):
            lo, hi = (len(pieces) * q) // n, (len(pieces) * (q + 1)) // n
            d(pieces[lo:hi])

    def gu_dots(b):
        ds = []
        for g in range(NG):
            def d(ps, g=g):
                hlf = len(ps) // 2
                gu(b, g, ps[:hlf], ps[hlf:])
            ds.append(d)
        return ds

    def dn_dots(b):
        return [functools.partial(down_tile, b, n) for n in range(D // 128)]

    def mix(a, b_):
        out = []
        n = len(a) + len(b_)
        ia = ib = 0
        for q in range(n):
            if ib >= len(b_) or (ia < len(a) and ia * len(b_) <= ib * len(a)):
                out.append(a[ia]); ia += 1
            else:
                out.append(b_[ib]); ib += 1
        return out

    def wait_wm(i): wait(("wm", i))
    def conv_phase():
        mod_done = set()
        for b in range(NB):
            if b == 0:
                wait("wf", "sk", "sd")
                setup()
            wait(("k", b), ("v", b), ("ssmk", b))
            todo = [i for i in range(5) if wm_after[i] < b and i not in mod_done]
            if todo:
                wait("c")
            for i in todo:
                wait_wm(i)
            ready0 = len(mod_done) + len(todo) == 5 and max(wm_after) < b and todo
            if ready0:
                wait(("x", 0))
            for i in todo:
                mod_piece(i); mod_done.add(i)
            for i in chunks(b):
                k_spec(i)
                x_spec(i)
            if b > 0 and b - 1 < PP:
                if b == 1:
                    wait("wi")
                for i in chunks(b - 1):
                    accum(i)
                for i in chunks(b - 1):
                    inv(i)
            if ready0:
                for i in chunks(0):
                    conv_out(i)
        todo = [i for i in range(5) if i not in mod_done]
        if todo:
            wait("c", ("x", 0))
            for i in todo:
                wait_wm(i)
            for i in todo:
                mod_piece(i)
        if PP == NB:
            for i in chunks(NB - 1):
                accum(i)
        if todo:
            for i in chunks(0):
                conv_out(i)
        if PP == NB:
            for i in chunks(NB - 1):
                inv(i)


    if BB:
        raise NotImplementedError
    else:
        conv_phase()

    late = {r: [] for r in range(NB)}
    R0 = int(os.environ.get("R0", "1"))
    wts = [float(a) for a in os.environ.get("RW", "1,1,1,1,1,1,1,1").split(",")]
    jobs = []
    for bb in range(PP, NB):
        ps = acc_pieces(bb)
        cost = (4 * bb + 3) / NSPL
        jobs += [(bb, p, cost) for p in ps]
    if jobs:
        rlast = NB - 3
        total = sum(j[2] for j in jobs)
        pos = 0
        for r in range(R0, rlast + 1):
            rem_w = sum(wts[R0:rlast + 1][r - R0:])
            rem_c = sum(j[2] for j in jobs[pos:])
            need = wts[r] / rem_w * rem_c
            for rr in range(r, rlast + 1):
                c_dl = sum(j[2] for j in jobs[pos:] if j[0] - 2 <= rr)
                need = max(need, wts[r] / sum(wts[r:rr + 1]) * c_dl)
            acc_c = 0
            while pos < len(jobs) and (acc_c < need - 1e-6 or jobs[pos][0] - 2 <= r):
                late[r].append(jobs[pos][1]); acc_c += jobs[pos][2]; pos += 1
        assert pos == len(jobs)
    if 'Z' in ABL:
        late = {r: [] for r in range(NB)}

    if STOP < 0:
        o_v[0:MB, :] = h2_scr[0][...]
        odma[0].start(); odma[0].wait()
        wait(*order)
        return
    nt = FG // 128
    for b in range(NB):
        if b > STOP:
            o_v[(b - 1) * MB:b * MB, :] = (hh_scr[b - 1][:, 0:D].astype(f32) + hh_scr[b - 1][:, D:2 * D].astype(f32) + hh_scr[b - 1][:, F - D:F].astype(f32)).astype(bf16)
            odma[b - 1].start()
            for bb in range(b):
                odma[bb].wait()
            wait(*order)
            return
        if b == 0:
            lp = ln_pieces(1)
            gd = gu_dots(0)
            for q in range(len(GW) - 1):
                g0, g1 = GW[q], GW[q + 1]
                wait(("wg", q), ("wu", q))
                if q == len(GW) - 2:
                    wait(("x", 1))
                    region(gd[g0:g1], lp)
                else:
                    region(gd[g0:g1], [])
        else:
            if b == 1:
                wait(("x", 2))
            if b == LAG + 1:
                wait(*[("x", bb) for bb in range(3, NB)])
            if b == 2 and LAG == 2:
                pass
            pieces = ln_pieces(b + 1) if (b + 1 < NB and not (LAG == 2 and b == 2)) else []
            if b + 1 >= PP and b + 1 < NB:
                for i in chunks(b + 1):
                    inv(i)
            if b < LAG:
                region(gu_dots(b), mix(pieces, late[b]))
            elif b == LAG:
                region(gu_dots(b), mix(pieces, late[b]))
                wait("wd")
                wait_wm(5)
                if LAG == 2:
                    wait(*[("x", bb) for bb in range(3, NB)])
                    pieces = ln_pieces(b + 1)
                else:
                    pieces = []
                mod_piece(5)
                region(dn_dots(0), pieces)
                odma[0].start()
            else:
                pieces = mix(pieces, late[b])
                n1 = ((len(pieces) * 1) // 3) * DNP
                region(dn_dots(b - LAG), pieces[:n1])
                region(gu_dots(b), pieces[n1:])
                odma[b - LAG].start()
    for b in range(NB - LAG, NB - 1):
        region(dn_dots(b), [])
        odma[b].start()
    if TAIL:
        otl = [pltpu.make_async_copy(o_v.at[rows(NB - 1), pl.ds(n * 128, 128)], o_hbm.at[rows(NB - 1), pl.ds(n * 128, 128)], osems.at[NB + n]) for n in range(D // 128)]
        for n in range(D // 128):
            down_tile(NB - 1, n)
            otl[n].start()
        for bb in range(NB - 1):
            odma[bb].wait()
        for n in range(D // 128):
            otl[n].wait()
    else:
        region(dn_dots(NB - 1), [])
        odma[NB - 1].start()
        for bb in range(NB):
            odma[bb].wait()


@jax.jit
def pallas_adaLN_cond__ssm_conv_h3__glu_gated_reglu__prompt_kernel(
    A_q, A_k, A_v, A_shift_k, A_ssm_k, A_ssm_D, B_x, B_W_gate, B_W_up, B_W_down, c, w_mod):
    f32, bf16 = jnp.float32, jnp.bfloat16
    ins = (A_q.reshape(S, D), A_k.reshape(S, D), A_v.reshape(S, D), A_shift_k.T, A_ssm_k, A_ssm_D.reshape(1, D),
      B_W_gate, B_W_up, B_W_down, c, w_mod, jnp.asarray(_WF, bf16), jnp.asarray(_WI, bf16))
    _tm = {4: (NC, D, C), 6: (F // 128, D, 128), 7: (F // 128, D, 128), 8: (D // 128, F, 128), 10: (6 * D // 128, D, 128)}
    out = pl.pallas_call(
        kernel,
        out_shape=jax.ShapeDtypeStruct((S, D), A_q.dtype),
        in_specs=[pl.BlockSpec(memory_space=pl.ANY)] * len(ins),
        out_specs=pl.BlockSpec(memory_space=pl.ANY),
        scratch_shapes=[pltpu.VMEM(a.shape, a.dtype) for n, a in enumerate(ins)] + [
            pltpu.VMEM((S, D), bf16),
            [pltpu.VMEM((NP * C, D), f32) for _ in range(NC)],
            [pltpu.VMEM((NP * C, D), f32) for _ in range(NC)],
            [pltpu.VMEM((2 * C, D), f32) for _ in range(NC)],
            ([pltpu.VMEM((2 * C, 2 * D), bf16) for _ in range(NC // 2)] if PAIR else [pltpu.VMEM((2 * C, D), bf16) for _ in range(NC)]),
            [pltpu.VMEM((C, D), f32) for _ in range(NC)],
            [pltpu.VMEM((MB, D), f32) for _ in range(NB)],
            [pltpu.VMEM((MB, D), bf16) for _ in range(NB)],
            [pltpu.VMEM((MB, F), bf16) for _ in range(NB)],
            pltpu.VMEM((8, D), f32),
            pltpu.VMEM((16, D), f32),
            pltpu.SemaphoreType.DMA((128,)),
            pltpu.SemaphoreType.DMA((NB + 8,)),
        ],
        compiler_params=pltpu.CompilerParams(vmem_limit_bytes=120 * 2**20),
    )(*ins)
    return out.reshape(1, S, D)
```

```python
import functools

import numpy as np
import jax
import jax.numpy as jnp
import jax.experimental.pallas as pl
import jax.experimental.pallas.tpu as pltpu

S, D, F = 2048, 640, 1536
KS = 4
EPS = 1e-5
C = 128
NC = S // C
MB = 256
NB = S // MB
CPB = MB // C
FG = 256
NG = F // FG
FT = 8
PP = 6
NSPL = 3
R0 = 2
GW = (0, 2, 4, NG)
WM_AFTER = (4, 5, 5, 6, 6)


def _dft_consts():
    j = np.arange(C, dtype=np.float64)[:, None]
    n = np.arange(C, dtype=np.float64)[None, :]
    ang = np.pi * (2 * j + 1) * n / (2 * C) * np.where(j % 2 == 0, 1.0, -1.0)
    wf = np.concatenate([np.cos(ang), -np.sin(ang)], axis=0)
    wi = np.concatenate([np.cos(ang).T, -np.sin(ang).T], axis=1) / C
    perm = np.concatenate([np.concatenate([np.arange(f, f + FT), C + np.arange(f, f + FT)])
                           for f in range(0, C, FT)])
    return wf.astype(np.float32), wi[:, perm].astype(np.float32)


_WF, _WI = _dft_consts()


def _ln(x):
    m = jnp.mean(x, axis=-1, keepdims=True)
    xc = x - m
    v = jnp.mean(xc * xc, axis=-1, keepdims=True)
    return xc * jax.lax.rsqrt(v + EPS)


def _kernel(x_hbm, k_hbm, v_hbm, sk_hbm, ssmk_hbm, sd_hbm, wg_hbm, wu_hbm, wd_hbm, c_hbm, wm_hbm,
            wf_hbm, wi_hbm, o_hbm,
            x_v, k_v, v_v, sk_v, ssmk_v, sd_v, wg_v, wu_v, wd_v, c_v, wm_v, wf_v, wi_v, o_v,
            g_scr, xs_scr, kr_scr, y_scr, yy_scr, x1_scr, h2_scr, hh_scr, mod_scr, taps_scr, sems, osems):
    f32, bf16, i32 = jnp.float32, jnp.bfloat16, jnp.int32

    def rows(b):
        return pl.ds(b * MB, MB)

    def chunks(b):
        return range(b * CPB, (b + 1) * CPB)

    dmas, order = {}, []

    def add(name, src, dst):
        dmas[name] = pltpu.make_async_copy(src, dst, sems.at[len(order)])
        order.append(name)

    def add_wm(i):
        add(("wm", i), wm_hbm.at[:, pl.ds(i * D, D)], wm_v.at[:, pl.ds(i * D, D)])

    def add_x(b):
        add(("x", b), x_hbm.at[rows(b), :], x_v.at[rows(b), :])

    add("wf", wf_hbm, wf_v)
    add("sk", sk_hbm, sk_v)
    add("sd", sd_hbm, sd_v)
    for b in range(NB):
        add(("k", b), k_hbm.at[rows(b), :], k_v.at[rows(b), :])
        add(("v", b), v_hbm.at[rows(b), :], v_v.at[rows(b), :])
        add(("ssmk", b), ssmk_hbm.at[:, rows(b)], ssmk_v.at[:, rows(b)])
        if b == 0:
            add("wi", wi_hbm, wi_v)
            add("c", c_hbm, c_v)
        for i in range(5):
            if WM_AFTER[i] == b:
                add_wm(i)
        if b == max(WM_AFTER):
            add_x(0)
    for q in range(len(GW) - 1):
        cs = pl.ds(GW[q] * FG, (GW[q + 1] - GW[q]) * FG)
        add(("wg", q), wg_hbm.at[:, cs], wg_v.at[:, cs])
        add(("wu", q), wu_hbm.at[:, cs], wu_v.at[:, cs])
    add_x(1)
    add_x(2)
    add("wd", wd_hbm, wd_v)
    add_wm(5)
    for b in range(3, NB):
        add_x(b)
    for name in order:
        dmas[name].start()
    waited = set()

    def wait(*names):
        for n in names:
            if n not in waited:
                dmas[n].wait()
                waited.add(n)

    odma = [pltpu.make_async_copy(o_v.at[rows(b), :], o_hbm.at[rows(b), :], osems.at[b])
            for b in range(NB - 1)]

    def mod_piece(i):
        cc = c_v[...].astype(f32)
        sc = jnp.broadcast_to((cc * jax.nn.sigmoid(cc)).astype(bf16), (16, D))
        r = jnp.dot(sc, wm_v[:, i * D:(i + 1) * D], preferred_element_type=f32)[0:1, :]
        if i in (1, 4):
            r = r + 1.0
        mod_scr[i:i + 1, :] = r

    def k_spec(m):
        km = jax.lax.dot_general(wf_v[...], ssmk_v[:, m * C:(m + 1) * C], (((1,), (1,)), ((), ())),
                                 preferred_element_type=f32)
        kre, kim = km[:C], km[C:]
        if m == 0:
            ga, gb = kre, kim
        else:
            kp = kr_scr[m - 1]
            ga = kre - kp[C:2 * C, :]
            gb = kim + kp[0:C, :]
        g_scr[m][0:C, :] = ga
        g_scr[m][C:2 * C, :] = gb
        g_scr[m][2 * C:3 * C, :] = ga + gb
        if m < NC - 1:
            kp = kr_scr[m]
            kp[0:C, :] = kre
            kp[C:2 * C, :] = kim

    def x_spec(i):
        r0 = i * C
        if i == 0:
            kw = jnp.concatenate([jnp.zeros((16, D), f32), k_v[0:C, :].astype(f32)], axis=0)
        else:
            kw = k_v[r0 - 16:r0 + C, :].astype(f32)
        ks = None
        for s in range(KS):
            term = kw[16 - s:16 - s + C, :] * taps_scr[s:s + 1, :]
            ks = term if ks is None else ks + term
        kv = ks * v_v[r0:r0 + C, :].astype(f32)
        yy_scr[i][...] = kv * taps_scr[8:9, :]
        xm = jnp.dot(wf_v[...], kv.astype(bf16), preferred_element_type=f32)
        xc, xd = xm[:C], xm[C:]
        xs_scr[i][0:C, :] = xc
        xs_scr[i][C:2 * C, :] = xd - xc
        xs_scr[i][2 * C:3 * C, :] = xc + xd

    def token(val):
        bits = pltpu.bitcast(val, i32)
        t = None
        for q in range(bits.shape[1] // 128):
            p = bits[:, q * 128:(q + 1) * 128]
            t = p if t is None else t | p
        return t

    def accum_parts(p, f0, l0, nsplit):
        i0, i1 = 2 * p, 2 * p + 1

        def ld(ref):
            return [ref[pl.ds(q * C + f0, FT), l0:l0 + 128] for q in range(3)]

        gc = {}

        def G(m):
            if m not in gc:
                gc[m] = ld(g_scr[m])
            return gc[m]

        acc = {i0: None, i1: None}
        js_all = list(range(i1 + 1))
        ns = min(nsplit, len(js_all))

        def part(k):
            for j in js_all[(len(js_all) * k) // ns:(len(js_all) * (k + 1)) // ns]:
                xj = ld(xs_scr[j])
                for i in (i0, i1):
                    if j > i:
                        continue
                    g = G(i - j)
                    pr = [xj[0] * g[2], g[0] * xj[1], g[1] * xj[2]]
                    acc[i] = pr if acc[i] is None else [a + b for a, b in zip(acc[i], pr)]
            if k < ns - 1:
                t = None
                for i in (i0, i1):
                    if acc[i] is not None:
                        bt = pltpu.bitcast(acc[i][0], i32)
                        t = bt if t is None else t | bt
                return t
            res = [(acc[i][0] - acc[i][2], acc[i][0] + acc[i][1]) for i in (i0, i1)]
            re = jnp.concatenate([res[0][0], res[1][0]], axis=1)
            im = jnp.concatenate([res[0][1], res[1][1]], axis=1)
            yv = jnp.concatenate([re, im], axis=0).astype(bf16)
            y_scr[p][pl.ds(2 * f0, 2 * FT), 2 * l0:2 * l0 + 256] = yv
            return token(yv)

        return [functools.partial(part, k) for k in range(ns)]

    def acc_pieces(b, nsplit):
        return [f for p in range(b * CPB // 2, (b + 1) * CPB // 2) for f0 in range(0, C, FT)
                for l0 in range(0, D, 128) for f in accum_parts(p, f0, l0, nsplit)]

    def inv(b):
        for p in range(b * CPB // 2, (b + 1) * CPB // 2):
            r = jnp.dot(wi_v[...], y_scr[p][...], preferred_element_type=f32)
            for q, i in enumerate((2 * p, 2 * p + 1)):
                rr = jnp.concatenate([r[:, 256 * t + 128 * q:256 * t + 128 * q + 128]
                                      for t in range(D // 128)], axis=1)
                yy_scr[i][...] = yy_scr[i][...] + rr

    def conv_out(b):
        for i in chunks(b):
            r0 = i * C
            lr = r0 % MB
            x = x_v[r0:r0 + C, :].astype(f32)
            h = _ln(x) * mod_scr[1:2, :] + mod_scr[0:1, :]
            x1 = x + mod_scr[2:3, :] * (h * yy_scr[i][...])
            x1_scr[b][lr:lr + C, :] = x1
            h2_scr[b][lr:lr + C, :] = (_ln(x1) * mod_scr[4:5, :] + mod_scr[3:4, :]).astype(bf16)

    rowctr = [0]

    def tie(w, pieces):
        if not pieces:
            return w
        K, N = w.shape
        pos = [(kt, ct) for kt in range(K // 128) for ct in range(N // 128)]
        byrow, used = {}, set()
        for q, p in enumerate(pieces):
            kt, ct = pos[(q * len(pos)) // len(pieces)]
            r = rowctr[0] % 8
            while (kt * 8 + r, ct) in used:
                r = (r + 1) % 8
            rowctr[0] += 1
            used.add((kt * 8 + r, ct))
            byrow.setdefault(kt * 8 + r, []).append((ct, p()))
        keep = jnp.abs(wf_v[0:16, :].astype(f32))[0:8] <= 2.0
        outr, prev = [], 0
        for r16 in sorted(byrow):
            r0 = r16 * 16
            if r0 > prev:
                outr.append(w[prev:r0])
            cols, pc = [], 0
            for ct, t in sorted(byrow[r16], key=lambda a: a[0]):
                c0 = ct * 128
                if c0 > pc:
                    cols.append(w[r0:r0 + 16, pc:c0])
                wb = pltpu.bitcast(w[r0:r0 + 16, c0:c0 + 128], i32)
                cols.append(pltpu.bitcast(jnp.where(keep, wb, t), bf16))
                pc = c0 + 128
            if pc < N:
                cols.append(w[r0:r0 + 16, pc:N])
            outr.append(cols[0] if len(cols) == 1 else jnp.concatenate(cols, axis=1))
            prev = r0 + 16
        if prev < K:
            outr.append(w[prev:K])
        return jnp.concatenate(outr, axis=0)

    def gu(b, g, pieces=()):
        hlf = len(pieces) // 2
        h = h2_scr[b][...]
        gt = jnp.dot(h, tie(wg_v[:, g * FG:(g + 1) * FG], pieces[:hlf]), preferred_element_type=f32)
        ut = jnp.dot(h, tie(wu_v[:, g * FG:(g + 1) * FG], pieces[hlf:]), preferred_element_type=f32)
        hh_scr[b][:, g * FG:(g + 1) * FG] = (jnp.maximum(gt, 0.0) * ut).astype(bf16)

    def gu_all(b, pieces=()):
        n = len(pieces)
        for g in range(NG):
            gu(b, g, pieces[(n * g) // NG:(n * (g + 1)) // NG])

    def down_tile(b, n):
        cs = slice(n * 128, (n + 1) * 128)
        out = jnp.dot(hh_scr[b][...], wd_v[:, cs], preferred_element_type=f32)
        o_v[b * MB:(b + 1) * MB, cs] = (x1_scr[b][:, cs] + mod_scr[5:6, cs] * out).astype(o_v.dtype)

    def down(b):
        for n in range(D // 128):
            down_tile(b, n)
        odma[b].start()

    mod_done = set()
    for b in range(NB):
        if b == 0:
            wait("wf", "sk", "sd")
            taps_scr[0:KS, :] = sk_v[...].astype(f32)
            taps_scr[8:9, :] = sd_v[...].astype(f32).reshape(1, D)
        wait(("k", b), ("v", b), ("ssmk", b))
        todo = [i for i in range(5) if WM_AFTER[i] < b and i not in mod_done]
        if todo:
            wait("c", *[("wm", i) for i in todo])
        first_ln = bool(todo) and len(mod_done) + len(todo) == 5
        if first_ln:
            wait(("x", 0))
        for i in todo:
            mod_piece(i)
            mod_done.add(i)
        for i in chunks(b):
            k_spec(i)
            x_spec(i)
        if 0 < b <= PP:
            if b == 1:
                wait("wi")
            for f in acc_pieces(b - 1, 1):
                f()
            inv(b - 1)
        if first_ln:
            conv_out(0)
    assert len(mod_done) == 5

    late = {r: [] for r in range(NB)}
    jobs = [(bb, f, (4 * bb + 3) / NSPL) for bb in range(PP, NB) for f in acc_pieces(bb, NSPL)]
    pos, rlast = 0, NB - 3
    for r in range(R0, rlast + 1):
        need = max(sum(j[2] for j in jobs[pos:] if j[0] - 2 <= rr) / (rr - r + 1)
                   for rr in range(r, rlast + 1))
        got = 0.0
        while pos < len(jobs) and (got < need - 1e-6 or jobs[pos][0] - 2 <= r):
            late[r].append(jobs[pos][1])
            got += jobs[pos][2]
            pos += 1
    assert pos == len(jobs)

    for q in range(len(GW) - 1):
        wait(("wg", q), ("wu", q))
        if q == len(GW) - 2:
            wait(("x", 1))
            conv_out(1)
        for g in range(GW[q], GW[q + 1]):
            gu(0, g)
    wait(("x", 2))
    conv_out(2)
    gu_all(1, late[1])
    gu_all(2, late[2])
    wait("wd", ("wm", 5))
    wait(*[("x", b) for b in range(3, NB)])
    conv_out(3)
    mod_piece(5)
    down(0)
    for b in range(3, NB):
        if PP <= b + 1 < NB:
            inv(b + 1)
        if b + 1 < NB:
            conv_out(b + 1)
        down(b - 2)
        gu_all(b, late[b])
    down(NB - 2)
    tail = [pltpu.make_async_copy(o_v.at[rows(NB - 1), pl.ds(n * 128, 128)],
                                  o_hbm.at[rows(NB - 1), pl.ds(n * 128, 128)], osems.at[NB + n])
            for n in range(D // 128)]
    for n in range(D // 128):
        down_tile(NB - 1, n)
        tail[n].start()
    for d in odma + tail:
        d.wait()


@jax.jit
def pallas_adaLN_cond__ssm_conv_h3__glu_gated_reglu__prompt_kernel(
    A_q, A_k, A_v, A_shift_k, A_ssm_k, A_ssm_D, B_x, B_W_gate, B_W_up, B_W_down, c, w_mod):
    f32, bf16 = jnp.float32, jnp.bfloat16
    ins = (A_q.reshape(S, D), A_k.reshape(S, D), A_v.reshape(S, D), A_shift_k.T, A_ssm_k, A_ssm_D,
           B_W_gate, B_W_up, B_W_down, c, w_mod, jnp.asarray(_WF, bf16), jnp.asarray(_WI, bf16))
    out = pl.pallas_call(
        _kernel,
        out_shape=jax.ShapeDtypeStruct((S, D), A_q.dtype),
        in_specs=[pl.BlockSpec(memory_space=pl.ANY)] * len(ins),
        out_specs=pl.BlockSpec(memory_space=pl.ANY),
        scratch_shapes=[pltpu.VMEM(a.shape, a.dtype) for a in ins] + [
            pltpu.VMEM((S, D), bf16),
            [pltpu.VMEM((3 * C, D), f32) for _ in range(NC)],
            [pltpu.VMEM((3 * C, D), f32) for _ in range(NC)],
            [pltpu.VMEM((2 * C, D), f32) for _ in range(NC)],
            [pltpu.VMEM((2 * C, 2 * D), bf16) for _ in range(NC // 2)],
            [pltpu.VMEM((C, D), f32) for _ in range(NC)],
            [pltpu.VMEM((MB, D), f32) for _ in range(NB)],
            [pltpu.VMEM((MB, D), bf16) for _ in range(NB)],
            [pltpu.VMEM((MB, F), bf16) for _ in range(NB)],
            pltpu.VMEM((8, D), f32),
            pltpu.VMEM((16, D), f32),
            pltpu.SemaphoreType.DMA((64,)),
            pltpu.SemaphoreType.DMA((NB + 8,)),
        ],
        compiler_params=pltpu.CompilerParams(vmem_limit_bytes=120 * 2**20),
    )(*ins)
    return out.reshape(1, S, D)
```
